```python
import jax
import jax.numpy as jnp

def _softmax(x, axis=-1):
    return jax.nn.softmax(x, axis=axis)
def _gelu(x):
    return jax.nn.gelu(x, approximate=True)
def _silu(x):
    return jax.nn.silu(x)
def _sigmoid(x):
    return jax.nn.sigmoid(x)
def _layernorm(x, axis=-1, eps=1e-5):
    m = jnp.mean(x, axis=axis, keepdims=True)
    v = jnp.var(x, axis=axis, keepdims=True)
    return (x - m) / jnp.sqrt(v + eps)
def _scatter_add(tgt, idx, src, axis=0):
    return tgt.at[idx].add(src)
def _segment_sum(src, seg, n):
    return jax.ops.segment_sum(src, seg, n)
class _Rng:
    def __init__(self, key):
        self._k = key
    def _next(self):
        self._k, sub = jax.random.split(self._k)
        return sub
    def normal(self, shape):
        return jax.random.normal(self._next(), shape, dtype=jnp.bfloat16)
    def randint(self, lo, hi, shape):
        return jax.random.randint(self._next(), shape, lo, hi, dtype=jnp.int32)
    def uniform(self, shape, lo=0.0, hi=1.0):
        return jax.random.uniform(self._next(), shape, jnp.bfloat16, lo, hi)
    def permutation(self, n):
        return jax.random.permutation(self._next(), n)


kernel_name = 'interleave_layers__sliding_block_cached__moe_arch_mod__decode'

def setup_inputs():
    _rng = _Rng(jax.random.key(int.from_bytes(__import__("os").urandom(4), "little")))
    _w = (lambda a: (lambda t: t.astype(jnp.bfloat16) if jnp.issubdtype(t.dtype, jnp.floating) else t)(jnp.asarray(a)))
    def _A_setup():
        B, Sq, D = 4, 1, 640
        Hq, Hkv, Sk, Dh = 32, 32, 4096, 192
        assert Hq % Hkv == 0, (Hq, Hkv)
        return {
            "x": _w((lambda *s: _rng.normal(s) * 0.05)(B, Sq, D)),
            "k_cache": _w((lambda *s: _rng.normal(s) * 0.05)(B, Hkv, Sk, Dh)),
            "v_cache": _w((lambda *s: _rng.normal(s) * 0.05)(B, Hkv, Sk, Dh)),
            "wq": _w((lambda *s: _rng.normal(s) * 0.05)(D, Hq * Dh) * (D ** -0.5)),
            "wo": _w((lambda *s: _rng.normal(s) * 0.05)(Hq * Dh, D) * ((Hq * Dh) ** -0.5)),
        }
    _A_in = _A_setup()

    def _B_setup():
        B, S, D, F, C = 4, 1, 640, 1536, 1
        return {
            "x": _w((lambda *s: _rng.normal(s) * 0.05)(B, S, D)),
            "w_r": _w((lambda *s: _rng.normal(s) * 0.05)(D)),
            "w_gate": _w((lambda *s: _rng.normal(s) * 0.05)(D, F)),
            "w_up": _w((lambda *s: _rng.normal(s) * 0.05)(D, F)),
            "w_down": _w((lambda *s: _rng.normal(s) * 0.05)(F, D)),
        }
    _B_in = _B_setup()

    return {
        "A_x": _A_in["x"],
        "A_k_cache": _A_in["k_cache"],
        "A_v_cache": _A_in["v_cache"],
        "A_wq": _A_in["wq"],
        "A_wo": _A_in["wo"],
        "B_x": _B_in["x"],
        "B_w_r": _B_in["w_r"],
        "B_w_gate": _B_in["w_gate"],
        "B_w_up": _B_in["w_up"],
        "B_w_down": _B_in["w_down"],
    }

def reference(A_x, A_k_cache, A_v_cache, A_wq, A_wo, B_x, B_w_r, B_w_gate, B_w_up, B_w_down):
    def _A_ref(x, k_cache, v_cache, wq, wo):
        B, Sq, D = x.shape
        Hq, Dh = 32, 192
        Hkv, Sk = k_cache.shape[1], k_cache.shape[2]
        W = min(4096, max(256, Sk // 4))
        rep = Hq // Hkv
        q = (lambda x, *d: x.transpose(*d))((x @ wq).reshape(B, Sq, Hq, Dh), 0, 2, 1, 3)
        k = jnp.repeat(k_cache[:, :, Sk - W:, :], rep, axis=1)
        v = jnp.repeat(v_cache[:, :, Sk - W:, :], rep, axis=1)
        scores = jnp.einsum("bhqd,bhkd->bhqk", q, k) * (Dh ** -0.5)
        p = _softmax(scores, axis=-1)
        o = jnp.einsum("bhqk,bhkd->bhqd", p, v)
        return (lambda x, *d: x.transpose(*d))(o, 0, 2, 1, 3).reshape(B, Sq, Hq * Dh) @ wo

    def _B_ref(x, w_r, w_gate, w_up, w_down):
        B, S, D = x.shape
        C = 1
        r = x @ w_r
        idx = jnp.argsort(-r, axis=-1)[:, :C]
        idx_e = jnp.repeat(idx.reshape(B, C, 1), D, axis=2)
        x_sel = jnp.take_along_axis(x, idx_e, axis=1)
        g = _silu(x_sel @ w_gate)
        u = x_sel @ w_up
        y = (g * u) @ w_down
        r_sel = _sigmoid(jnp.take_along_axis(r, idx, axis=1))
        y = y * r_sel.reshape(B, C, 1)
        b_off = (jnp.arange(B) * S).reshape(B, 1)
        flat_idx = (idx + b_off).reshape(B * C)
        zero = (x * 0.0).reshape(B * S, D)
        upd = _scatter_add(zero, flat_idx, y.reshape(B * C, D), axis=0)
        return x + upd.reshape(B, S, D)

    x = A_x
    x = x + _A_ref(_layernorm(x, axis=-1), A_k_cache, A_v_cache, A_wq, A_wo)
    x = x + _B_ref(_layernorm(x, axis=-1), B_w_r, B_w_gate, B_w_up, B_w_down)
    x = x + _A_ref(_layernorm(x, axis=-1), A_k_cache, A_v_cache, A_wq, A_wo)
    x = x + _B_ref(_layernorm(x, axis=-1), B_w_r, B_w_gate, B_w_up, B_w_down)
    return x
```

```python
import jax
import jax.numpy as jnp
import jax.experimental.pallas as pl
import jax.experimental.pallas.tpu as pltpu
from jax import lax

B, D = 4, 640
H, DH, SK = 32, 192, 4096
W = min(4096, max(256, SK // 4))
F = 1536
HD = H * DH
G = 8
NG = H // G
GW = G * DH
EPS = 1e-5
BF = jnp.bfloat16
F32 = jnp.float32
I32 = jnp.int32


def _layernorm(x):
    m = jnp.mean(x, axis=1, keepdims=True)
    d = x - m
    v = jnp.mean(d * d, axis=1, keepdims=True)
    return d / jnp.sqrt(v + EPS)


def _bf(ref_slice):
    return pltpu.bitcast(ref_slice, BF)


def _kernel(x_hbm, k_hbm, v_hbm, wq_hbm, wo_hbm, wr_hbm, wg_hbm, wu_hbm, wd_hbm,
            o_ref,
            x_s, wr_s, k_s, v_s, wq_s, wo_s, wg_s, wu_s, wd_s,
            sem_small, sem_k, sem_v, sem_wq, sem_wo, sem_ffn):
    k32 = k_hbm.bitcast(I32)
    v32 = v_hbm.bitcast(I32)
    wq32 = wq_hbm.bitcast(I32)
    wo32 = wo_hbm.bitcast(I32)

    def k_copy(b, g):
        r0 = b * (HD // 2) + g * (GW // 2)
        if not isinstance(r0, int):
            r0 = pl.multiple_of(r0, GW // 2)
        return pltpu.make_async_copy(
            k32.at[pl.ds(r0, GW // 2), pl.ds(SK - W, W)], k_s.at[b, g], sem_k.at[b, g])

    def v_copy(b, g):
        r0 = b * (HD // 2) + g * (GW // 2)
        if not isinstance(r0, int):
            r0 = pl.multiple_of(r0, GW // 2)
        return pltpu.make_async_copy(
            v32.at[pl.ds(r0, GW // 2), pl.ds(SK - W, W)], v_s.at[b, g], sem_v.at[b, g])

    def wq_copy(g):
        return pltpu.make_async_copy(
            wq32.at[:, pl.ds(g * GW, GW)], wq_s.at[g], sem_wq.at[g])

    def wo_copy(g):
        return pltpu.make_async_copy(
            wo32.at[pl.ds(g * (GW // 2), GW // 2), :], wo_s.at[g], sem_wo.at[g])

    x_copy = pltpu.make_async_copy(x_hbm, x_s, sem_small.at[0])
    wr_copy = pltpu.make_async_copy(wr_hbm, wr_s, sem_small.at[1])
    wg_copy = pltpu.make_async_copy(wg_hbm.bitcast(I32), wg_s, sem_ffn.at[0])
    wu_copy = pltpu.make_async_copy(wu_hbm.bitcast(I32), wu_s, sem_ffn.at[1])
    wd_copy = pltpu.make_async_copy(wd_hbm.bitcast(I32), wd_s, sem_ffn.at[2])

    for g in range(NG):
        wq_copy(g).start()
        if g == 0:
            x_copy.start()
            wr_copy.start()
        k_copy(0, g).start()
    for g in range(NG):
        v_copy(0, g).start()
        wo_copy(g).start()
    wg_copy.start()
    wu_copy.start()
    wd_copy.start()

    row = lax.broadcasted_iota(I32, (G, GW), 0)
    col = lax.broadcasted_iota(I32, (G, GW), 1)
    mask = (col >= row * DH) & (col < row * DH + DH)
    row8 = lax.broadcasted_iota(I32, (8, D), 0)
    scale = DH ** -0.5

    x_copy.wait()
    wr_copy.wait()
    x_all = x_s[...].astype(F32)
    wr = wr_s[...].astype(F32)
    row4 = lax.broadcasted_iota(I32, (B, D), 0)

    def attention(b, xn, first):
        acc = jnp.zeros((G, D), F32)
        for g in range(NG):
            if first:
                if g < NG:
                    @pl.when(b == 0)
                    def _():
                        wq_copy(g).wait()
            q = jnp.dot(xn, _bf(wq_s[g]), preferred_element_type=F32)
            qbd = jnp.where(mask, q, 0.0).astype(BF)
            if first:
                k_copy(b, g).wait()

                @pl.when(b + 1 < B)
                def _():
                    k_copy(b + 1, g).start()
            s = jnp.dot(qbd, _bf(k_s[b, g]), preferred_element_type=F32) * scale
            m = jnp.max(s, axis=1, keepdims=True)
            p = jnp.exp(s - m)
            l = jnp.sum(p, axis=1, keepdims=True)
            if first:
                v_copy(b, g).wait()

                @pl.when(b + 1 < B)
                def _():
                    v_copy(b + 1, g).start()

                @pl.when(b == 0)
                def _():
                    wo_copy(g).wait()
            o = lax.dot_general(p.astype(BF), _bf(v_s[b, g]), (((1,), (1,)), ((), ())),
                                preferred_element_type=F32)
            o = jnp.where(mask, o * (1.0 / l), 0.0).astype(BF)
            acc = acc + jnp.dot(o, _bf(wo_s[g]), preferred_element_type=F32)
        return jnp.broadcast_to(jnp.sum(acc, axis=0, keepdims=True), (8, D))

    def ffn(xn_f32):
        xn = xn_f32.astype(BF)
        r = jnp.sum(xn.astype(F32) * wr, axis=1, keepdims=True)
        gate = jnp.dot(xn, _bf(wg_s[...]), preferred_element_type=F32)
        up = jnp.dot(xn, _bf(wu_s[...]), preferred_element_type=F32)
        h = (gate * jax.nn.sigmoid(gate) * up).astype(BF)
        y = jnp.dot(h, _bf(wd_s[...]), preferred_element_type=F32)
        return xn.astype(F32) + y * jax.nn.sigmoid(r)

    def per_batch(b, out):
        x = jnp.broadcast_to(
            jnp.sum(jnp.where(row4 == b, x_all, 0.0), axis=0, keepdims=True), (8, D))
        x = x + attention(b, _layernorm(x).astype(BF), True)

        @pl.when(b == 0)
        def _():
            wg_copy.wait()
            wu_copy.wait()
            wd_copy.wait()
        x = x + ffn(_layernorm(x))
        x = x + attention(b, _layernorm(x).astype(BF), False)
        x = x + ffn(_layernorm(x))
        return jnp.where(row8 == b, x, out)

    out = lax.fori_loop(0, B, per_batch, jnp.zeros((8, D), F32))
    o_ref[...] = out[0:B].astype(BF)


@jax.jit
def pallas_interleave_layers__sliding_block_cached__moe_arch_mod__decode_kernel(
    A_x: jax.Array,
    A_k_cache: jax.Array,
    A_v_cache: jax.Array,
    A_wq: jax.Array,
    A_wo: jax.Array,
    B_x: jax.Array,
    B_w_r: jax.Array,
    B_w_gate: jax.Array,
    B_w_up: jax.Array,
    B_w_down: jax.Array,
):
    kT = jnp.swapaxes(A_k_cache, 2, 3).reshape(B * HD, SK)
    vT = jnp.swapaxes(A_v_cache, 2, 3).reshape(B * HD, SK)
    x2 = A_x.reshape(B, D)
    wr2 = B_w_r.reshape(1, D)

    any_spec = pl.BlockSpec(memory_space=pl.ANY)
    out = pl.pallas_call(
        _kernel,
        out_shape=jax.ShapeDtypeStruct((B, D), BF),
        in_specs=[any_spec] * 9,
        out_specs=pl.BlockSpec(memory_space=pltpu.VMEM),
        scratch_shapes=[
            pltpu.VMEM((B, D), BF),
            pltpu.VMEM((1, D), BF),
            pltpu.VMEM((B, NG, GW // 2, W), I32),
            pltpu.VMEM((B, NG, GW // 2, W), I32),
            pltpu.VMEM((NG, D // 2, GW), I32),
            pltpu.VMEM((NG, GW // 2, D), I32),
            pltpu.VMEM((D // 2, F), I32),
            pltpu.VMEM((D // 2, F), I32),
            pltpu.VMEM((F // 2, D), I32),
            pltpu.SemaphoreType.DMA((2,)),
            pltpu.SemaphoreType.DMA((B, NG)),
            pltpu.SemaphoreType.DMA((B, NG)),
            pltpu.SemaphoreType.DMA((NG,)),
            pltpu.SemaphoreType.DMA((NG,)),
            pltpu.SemaphoreType.DMA((3,)),
        ],
        compiler_params=pltpu.CompilerParams(vmem_limit_bytes=127 * 1024 * 1024),
    )(x2, kT, vT, A_wq, A_wo, wr2, B_w_gate, B_w_up, B_w_down)
    return out.reshape(B, 1, D)
```

```python
import itertools
import jax
import jax.numpy as jnp
import jax.experimental.pallas as pl
import jax.experimental.pallas.tpu as pltpu
from jax import lax

B, D = 4, 640
H, DH, SK = 32, 192, 4096
W = min(4096, max(256, SK // 4))
F = 1536
HD = H * DH
G = 8
NG = H // G
GW = G * DH
GR = GW // 2
UW = 2 * DH
UR = UW // 2
NU = H // 2
EPS = 1e-5
BF = jnp.bfloat16
F32 = jnp.float32
I32 = jnp.int32
SCALE = DH ** -0.5
SKEW = 1
VB = 6
QN = 4


def _layernorm(x):
    m = jnp.mean(x, axis=1, keepdims=True)
    d = x - m
    v = jnp.mean(d * d, axis=1, keepdims=True)
    return d / jnp.sqrt(v + EPS)


def _bf(x):
    return pltpu.bitcast(x, BF)


def _kernel(x_hbm, k_hbm, v_hbm, wq_hbm, wo_hbm, wr_hbm, wg_hbm, wu_hbm, wd_hbm,
            o_ref,
            x_s, wr_s, k_s, v_s, wq_s, wo_s, wg_s, wu_s, wd_s,
            sem_w, sem_k, sem_v):
    k32 = k_hbm.bitcast(I32)
    v32 = v_hbm.bitcast(I32)

    def k_copy(b, g):
        r0 = b * (HD // 2) + g * GR
        if not isinstance(r0, int):
            r0 = pl.multiple_of(r0, GR)
        return pltpu.make_async_copy(
            k32.at[pl.ds(r0, GR), pl.ds(SK - W, W)], k_s.at[b, pl.ds(g * GR, GR)], sem_k.at[b, g])

    def v_copy(b, u):
        r0 = b * (HD // 2) + u * UR
        if not isinstance(r0, int):
            r0 = pl.multiple_of(r0, UR)
        return pltpu.make_async_copy(
            v32.at[pl.ds(r0, UR), pl.ds(SK - W, W)], v_s.at[b, pl.ds(u * UR, UR)], sem_v.at[b, u])

    def start_batch(b):
        for g in range(NG):
            k_copy(b, g).start()
            for uu in range(G // 2):
                v_copy(b, g * (G // 2) + uu).start()

    w_copies = [
        pltpu.make_async_copy(wq_hbm.bitcast(I32), wq_s, sem_w.at[0]),
        pltpu.make_async_copy(x_hbm, x_s, sem_w.at[1]),
        pltpu.make_async_copy(wr_hbm, wr_s, sem_w.at[2]),
        pltpu.make_async_copy(wo_hbm.bitcast(I32), wo_s, sem_w.at[3]),
        pltpu.make_async_copy(wg_hbm.bitcast(I32), wg_s, sem_w.at[4]),
        pltpu.make_async_copy(wu_hbm.bitcast(I32), wu_s, sem_w.at[5]),
        pltpu.make_async_copy(wd_hbm.bitcast(I32), wd_s, sem_w.at[6]),
    ]
    for c in w_copies:
        c.start()
    start_batch(0)

    row = lax.broadcasted_iota(I32, (8, GW), 0)
    col = lax.broadcasted_iota(I32, (8, GW), 1)
    mask = (col >= row * DH) & (col < row * DH + DH)
    r8 = lax.broadcasted_iota(I32, (8, 128), 0)
    c8 = lax.broadcasted_iota(I32, (8, 128), 1)
    lidx = c8 - 2 * r8
    row8 = lax.broadcasted_iota(I32, (8, D), 0)
    row4 = lax.broadcasted_iota(I32, (B, D), 0)

    for c in w_copies:
        c.wait()
    x_all = x_s[...].astype(F32)
    wr = wr_s[...].reshape(1, D).astype(F32)

    def attention_stream(b, xn):
        acc = jnp.zeros((8, D), F32)
        for g in range(NG):
            q = jnp.dot(xn, _bf(wq_s[:, g * GW:(g + 1) * GW]), preferred_element_type=F32)
            qbd = jnp.where(mask, q, 0.0).astype(BF)
            k_copy(b, g).wait()
            s = jnp.dot(qbd, _bf(k_s[b, g * GR:(g + 1) * GR, :]), preferred_element_type=F32) * SCALE
            m = jnp.max(s, axis=1, keepdims=True)
            p = jnp.exp(s - m)
            l = jnp.sum(p, axis=1, keepdims=True)
            pn = (p * (1.0 / l)).astype(BF)
            for uu in range(G // 2):
                u = g * (G // 2) + uu
                v_copy(b, u).wait()
                o = lax.dot_general(pn, _bf(v_s[b, u * UR:(u + 1) * UR, :]), (((1,), (1,)), ((), ())),
                                    preferred_element_type=F32)
                o = jnp.where(mask[:, uu * UW:(uu + 1) * UW], o, 0.0).astype(BF)
                acc = acc + jnp.dot(o, _bf(wo_s[u * UR:(u + 1) * UR, :]), preferred_element_type=F32)
        return jnp.broadcast_to(jnp.sum(acc, axis=0, keepdims=True), (8, D))

    def attention_resident(b, xn):
        ZM = []

        def tok():
            return ZM[-1 - SKEW] * 0.0 if len(ZM) > SKEW else None

        def q_gen(g, out):
            qt = []
            for t in range(0, GW // 128, QN):
                d = jnp.dot(xn, _bf(wq_s[:, g * GW + t * 128:g * GW + (t + QN) * 128]),
                            preferred_element_type=F32)
                qt.append(d)
                ZM.append(d[:, 0:128])
                yield QN * 5
            out.append(jnp.where(mask, jnp.concatenate(qt, axis=1), 0.0).astype(BF))

        def s_gen(g, qsrc, out):
            st = []
            for j in range(W // 128):
                d = jnp.dot(qsrc[0], _bf(k_s[b, g * GR:(g + 1) * GR, j * 128:(j + 1) * 128]),
                            preferred_element_type=F32)
                st.append(d)
                ZM.append(d)
                yield GW // 128
            s = jnp.concatenate(st, axis=1) * SCALE
            m = jnp.max(s, axis=1, keepdims=True)
            p = jnp.exp(s - m)
            l = jnp.sum(p, axis=1, keepdims=True)
            out.append(p * (1.0 / l))

        def o_gen(g, o, out):
            ot = []
            for n in range(D // 128):
                d = jnp.dot(o, _bf(wo_s[g * GR:(g + 1) * GR, n * 128:(n + 1) * 128]),
                            preferred_element_type=F32)
                ot.append(d)
                ZM.append(d)
                yield GW // 128
            out.append(jnp.concatenate(ot, axis=1))

        def pv_gen(g, pn, out):
            tiles = [jnp.zeros((8, 128), F32) for _ in range(GW // 128)]
            for h in range(G):
                pb = jnp.broadcast_to(pn[h:h + 1, :], (8, W))
                pj0 = [pb[:, j * 128:(j + 1) * 128] for j in range(W // 128)]
                for i0 in range(0, DH // 16, VB):
                    z = tok()
                    pj = pj0 if z is None else [p + z for p in pj0]
                    for i in range(i0, i0 + VB):
                        r0 = g * GR + h * (DH // 2) + i * 8
                        for j in range(W // 128):
                            w = v_s[b, r0:r0 + 8, j * 128:(j + 1) * 128]
                            lo = pltpu.bitcast(w << 16, F32) * pj[j]
                            hi = pltpu.bitcast(w & jnp.int32(-65536), F32) * pj[j]
                            if j == 0:
                                a_lo, a_hi = lo, hi
                            else:
                                a_lo, a_hi = a_lo + lo, a_hi + hi
                        rlo = jnp.sum(a_lo, axis=1, keepdims=True)
                        rhi = jnp.sum(a_hi, axis=1, keepdims=True)
                        rg = h * DH + i * 16
                        t, off = rg // 128, rg % 128
                        tl = jnp.where(lidx == off, rlo, tiles[t])
                        tiles[t] = jnp.where(lidx == off + 1, rhi, tl)
                    yield VB
            out.append(jnp.concatenate(tiles, axis=1).astype(BF))

        def interleave(ga, gb, na, nb):
            a = itertools.chain(*ga)
            done_a = not ga
            done_b = gb is None
            ia = ib = 0
            while not (done_a and done_b):
                if not done_a and (done_b or ia * nb <= ib * na):
                    try:
                        ia += next(a)
                    except StopIteration:
                        done_a = True
                else:
                    try:
                        ib += next(gb)
                    except StopIteration:
                        done_b = True

        acc = jnp.zeros((8, D), F32)
        ps, os_ = {}, {}
        T = GW // 128
        for per in range(-1, NG + 1):
            ga, na = [], 0
            o1, o2, o3, o4 = [], [], [], []
            if 0 <= per + 1 < NG:
                ga.append(q_gen(per + 1, o1))
                ga.append(s_gen(per + 1, o1, o2))
                na += 13 * T
            if 0 <= per - 1 < NG:
                ga.append(o_gen(per - 1, os_.pop(per - 1), o3))
                na += 5 * T
            gb = pv_gen(per, ps.pop(per), o4) if 0 <= per < NG else None
            interleave(ga, gb, max(na, 1), G * 12)
            if o2:
                ps[per + 1] = o2[0]
            if o3:
                acc = acc + o3[0]
            if o4:
                os_[per] = o4[0]
        return jnp.broadcast_to(jnp.sum(acc, axis=0, keepdims=True), (8, D))

    def ffn(xn_f32):
        xn = xn_f32.astype(BF)
        r = jnp.sum(xn.astype(F32) * wr, axis=1, keepdims=True)
        gate = jnp.dot(xn, _bf(wg_s[...]), preferred_element_type=F32)
        up = jnp.dot(xn, _bf(wu_s[...]), preferred_element_type=F32)
        h = (gate * jax.nn.sigmoid(gate) * up).astype(BF)
        y = jnp.dot(h, _bf(wd_s[...]), preferred_element_type=F32)
        return xn.astype(F32) + y * jax.nn.sigmoid(r)

    def per_batch(b, out):
        @pl.when(b + 1 < B)
        def _():
            start_batch(b + 1)
        x = jnp.broadcast_to(
            jnp.sum(jnp.where(row4 == b, x_all, 0.0), axis=0, keepdims=True), (8, D))
        x = x + attention_stream(b, _layernorm(x).astype(BF))
        x = x + ffn(_layernorm(x))
        x = x + attention_resident(b, _layernorm(x).astype(BF))
        x = x + ffn(_layernorm(x))
        return jnp.where(row8 == b, x, out)

    out = lax.fori_loop(0, B, per_batch, jnp.zeros((8, D), F32))
    o_ref[...] = out[0:B].astype(BF)


@jax.jit
def pallas_interleave_layers__sliding_block_cached__moe_arch_mod__decode_kernel(
    A_x, A_k_cache, A_v_cache, A_wq, A_wo, B_x, B_w_r, B_w_gate, B_w_up, B_w_down,
):
    kT = jnp.swapaxes(A_k_cache, 2, 3).reshape(B * HD, SK)
    vT = jnp.swapaxes(A_v_cache, 2, 3).reshape(B * HD, SK)
    x2 = A_x.reshape(B, D)
    any_spec = pl.BlockSpec(memory_space=pl.ANY)
    out = pl.pallas_call(
        _kernel,
        out_shape=jax.ShapeDtypeStruct((B, D), BF),
        in_specs=[any_spec] * 9,
        out_specs=pl.BlockSpec(memory_space=pltpu.VMEM),
        scratch_shapes=[
            pltpu.VMEM((B, D), BF),
            pltpu.VMEM((D,), BF),
            pltpu.VMEM((B, HD // 2, W), I32),
            pltpu.VMEM((B, HD // 2, W), I32),
            pltpu.VMEM((D // 2, HD), I32),
            pltpu.VMEM((HD // 2, D), I32),
            pltpu.VMEM((D // 2, F), I32),
            pltpu.VMEM((D // 2, F), I32),
            pltpu.VMEM((F // 2, D), I32),
            pltpu.SemaphoreType.DMA((7,)),
            pltpu.SemaphoreType.DMA((B, NG)),
            pltpu.SemaphoreType.DMA((B, NU)),
        ],
        compiler_params=pltpu.CompilerParams(vmem_limit_bytes=127 * 1024 * 1024),
    )(x2, kT, vT, A_wq, A_wo, B_w_r, B_w_gate, B_w_up, B_w_down)
    return out.reshape(B, 1, D)
```

```python
import itertools
import jax
import jax.numpy as jnp
import jax.experimental.pallas as pl
import jax.experimental.pallas.tpu as pltpu
from jax import lax

B, D = 4, 640
H, DH, SK = 32, 192, 4096
W = min(4096, max(256, SK // 4))
F = 1536
HD = H * DH
G = 8
NG = H // G
GW = G * DH
GR = GW // 2
UW = 2 * DH
UR = UW // 2
NU = H // 2
EPS = 1e-5
BF = jnp.bfloat16
F32 = jnp.float32
I32 = jnp.int32
SCALE = DH ** -0.5
SKEW = int(1)
VB = int(6)
QN = int(4)
SN = int(1)
ON = int(1)
LAG = int(1)
NS = int(2)
NF = int(30)
WV = int(8)
GATE = int(2)
SKM = int(-1)
FWV = int(0)
UB = int(32)
LN1P = int(1)
SPLIT = int(1)
ROLL = 0
def _chunks(s):
    c = [int(x) for x in s.split('_')]
    return list(zip(c[:-1], c[1:]))
KC = _chunks('0_8_16_24_32')
VC = _chunks('0_8_16_24_26_28_30_31_32')
DMA_ORDER = sorted([('k', i) for i in range(len(KC))] + [('v', i) for i in range(len(VC))],
                   key=lambda t: ((KC if t[0] == 'k' else VC)[t[1]][0] // G, t[0], t[1])) if int(1) else \
    [('k', i) for i in range(len(KC))] + [('v', i) for i in range(len(VC))]
GS = [int(c) for c in '88862']
MX = [int(c) for c in '4']


def _layernorm(x):
    if LN1P:
        m = jnp.sum(x, axis=1, keepdims=True) * (1.0 / D)
        v = jnp.sum(x * x, axis=1, keepdims=True) * (1.0 / D) - m * m
        return (x - m) * lax.rsqrt(jnp.maximum(v, 0.0) + EPS)
    m = jnp.mean(x, axis=1, keepdims=True)
    d = x - m
    v = jnp.mean(d * d, axis=1, keepdims=True)
    return d / jnp.sqrt(v + EPS)


def _bf(x):
    return pltpu.bitcast(x, BF)


def _kernel(x_hbm, k_hbm, v_hbm, wq_hbm, wo_hbm, wr_hbm, wg_hbm, wu_hbm, wd_hbm,
            o_ref,
            x_s, wr_s, k_s, v_s, vf_s, wq_s, wo_s, wg_s, wu_s, wd_s,
            sem_w, sem_k, sem_v):
    k32 = k_hbm.bitcast(I32)
    v32 = v_hbm.bitcast(I32)

    def kv_copy(src32, dst, sems, b, ci, h0, h1):
        r0, nr = h0 * (DH // 2), (h1 - h0) * (DH // 2)
        g0 = b * (HD // 2) + r0
        if not isinstance(g0, int):
            g0 = pl.multiple_of(g0, DH // 2)
        return pltpu.make_async_copy(
            src32.at[pl.ds(g0, nr), pl.ds(SK - W, W)], dst.at[b % NS, pl.ds(r0, nr)], sems.at[b, ci])

    def k_copy(b, ci):
        return kv_copy(k32, k_s, sem_k, b, ci, *KC[ci])

    def v_copy(b, ci):
        return kv_copy(v32, v_s, sem_v, b, ci, *VC[ci])

    def start_batch(b):
        for kind, ci in DMA_ORDER:
            (k_copy if kind == "k" else v_copy)(b, ci).start()

    w_copies = [
        pltpu.make_async_copy(wq_hbm.bitcast(I32), wq_s, sem_w.at[0]),
        pltpu.make_async_copy(x_hbm, x_s, sem_w.at[1]),
        pltpu.make_async_copy(wr_hbm, wr_s, sem_w.at[2]),
        pltpu.make_async_copy(wo_hbm.bitcast(I32), wo_s, sem_w.at[3]),
        pltpu.make_async_copy(wg_hbm.bitcast(I32), wg_s, sem_w.at[4]),
        pltpu.make_async_copy(wu_hbm.bitcast(I32), wu_s, sem_w.at[5]),
        pltpu.make_async_copy(wd_hbm.bitcast(I32), wd_s, sem_w.at[6]),
    ]
    for c in w_copies:
        c.start()
    start_batch(0)

    row = lax.broadcasted_iota(I32, (8, GW), 0)
    col = lax.broadcasted_iota(I32, (8, GW), 1)
    mask = (col >= row * DH) & (col < row * DH + DH)
    r8 = lax.broadcasted_iota(I32, (8, 128), 0)
    c8 = lax.broadcasted_iota(I32, (8, 128), 1)
    lidx = c8 - 2 * r8
    row8 = lax.broadcasted_iota(I32, (8, D), 0)
    row4 = lax.broadcasted_iota(I32, (B, D), 0)

    for c in w_copies:
        c.wait()
    x_all = x_s[...].astype(F32)
    wr = wr_s[...].reshape(1, D).astype(F32)

    def attention_stream(b, xn):
        sl = b % NS
        acc = jnp.zeros((8, D), F32)
        kw, vw = set(), set()

        def need(kind, h):
            chunks, done, cp = (KC, kw, k_copy) if kind == "k" else (VC, vw, v_copy)
            for ci, (h0, h1) in enumerate(chunks):
                if h0 <= h < h1 and ci not in done:
                    cp(b, ci).wait()
                    done.add(ci)

        def scores(g):
            q = jnp.dot(xn, _bf(wq_s[:, g * GW:(g + 1) * GW]), preferred_element_type=F32)
            qbd = jnp.where(mask, q, 0.0).astype(BF)
            need("k", g * G + G - 1)
            s = jnp.dot(qbd, _bf(k_s[sl, g * GR:(g + 1) * GR, :]), preferred_element_type=F32) * SCALE
            m = jnp.max(s, axis=1, keepdims=True)
            p = jnp.exp(s - m)
            l = jnp.sum(p, axis=1, keepdims=True)
            return (p * (1.0 / l)).astype(BF)

        pns = {}
        for g in range(NG):
            if g not in pns:
                ci = [i for i, (h0, h1) in enumerate(KC) if h0 <= g * G < h1][0]
                for g2 in range(g, NG):
                    if KC[ci][0] <= g2 * G < KC[ci][1]:
                        pns[g2] = scores(g2)
            pn = pns.pop(g)
            h = g * G
            while h < (g + 1) * G:
                ci = [i for i, (h0, h1) in enumerate(VC) if h0 <= h < h1][0]
                nh = min(2, VC[ci][1] - h)
                need("v", h)
                r0, nr = h * (DH // 2), nh * (DH // 2)
                o = lax.dot_general(pn, _bf(v_s[sl, r0:r0 + nr, :]), (((1,), (1,)), ((), ())),
                                    preferred_element_type=F32)
                c0 = (h - g * G) * DH
                if nh == 2:
                    msk = mask[:, c0:c0 + nh * DH]
                else:
                    msk = lax.broadcasted_iota(I32, (8, DH), 0) == (h - g * G)
                o = jnp.where(msk, o, 0.0).astype(BF)
                acc = acc + jnp.dot(o, _bf(wo_s[r0:r0 + nr, :]), preferred_element_type=F32)
                h += nh
                if h == VC[ci][1] and VC[ci][0] < NF:
                    u0, u1 = VC[ci][0] * (DH // 2) // UB, min(VC[ci][1], NF) * (DH // 2) // UB

                    def widen(i, c):
                        r = pl.multiple_of(i * UB, UB)
                        w = v_s[sl, pl.ds(r, UB), :]
                        vf_s[0, pl.ds(r, UB), :] = pltpu.bitcast(w << 16, F32)
                        vf_s[1, pl.ds(r, UB), :] = pltpu.bitcast(w & jnp.int32(-65536), F32)
                        return c
                    lax.fori_loop(u0, u1, widen, 0)
        return jnp.broadcast_to(jnp.sum(acc, axis=0, keepdims=True), (8, D))

    def attention_resident(b, xn):
        sl = b % NS
        ZM = []
        ng = len(GS)
        h0 = [sum(GS[:i]) for i in range(ng)]

        def tok():
            return ZM[-1 - SKEW] * 0.0 if (SKEW >= 0 and len(ZM) > SKEW) else None

        ZV = []

        FORCE = []

        def gate(lhs):
            if FORCE:
                z = FORCE.pop() * 0.0
                return (lhs.astype(F32) + jnp.concatenate([z] * (lhs.shape[1] // 128), axis=1)).astype(BF)
            if SKM < 0 or len(ZV) <= SKM:
                return lhs
            z = ZV[-1 - SKM] * 0.0
            return (lhs.astype(F32) + jnp.concatenate([z] * (lhs.shape[1] // 128), axis=1)).astype(BF)

        def gmask(g):
            n = GS[g] * DH
            row = lax.broadcasted_iota(I32, (8, n), 0)
            col = lax.broadcasted_iota(I32, (8, n), 1)
            return (col >= row * DH) & (col < row * DH + DH)

        def q_gen(g, out):
            nt = GS[g] * DH // 128
            c0 = h0[g] * DH
            qt = []
            t = 0
            while t < nt:
                n = min(QN, nt - t)
                d = jnp.dot(gate(xn), _bf(wq_s[:, c0 + t * 128:c0 + (t + n) * 128]), preferred_element_type=F32)
                qt.append(d)
                ZM.append(d[:, 0:128])
                t += n
                yield n * 5
            out.append(jnp.where(gmask(g), jnp.concatenate(qt, axis=1), 0.0).astype(BF))

        def s_gen(g, qsrc, out):
            r0, nr = h0[g] * DH // 2, GS[g] * DH // 2
            sn = max(1, SN * 8 // GS[g])
            st = []
            for j in range(0, W // 128, sn):
                d = jnp.dot(gate(qsrc[0]), _bf(k_s[sl, r0:r0 + nr, j * 128:(j + sn) * 128]),
                            preferred_element_type=F32)
                st.append(d)
                ZM.append(d[:, 0:128])
                yield sn * (GS[g] * DH // 128)
            s = jnp.concatenate(st, axis=1) * SCALE
            m = jnp.max(s, axis=1, keepdims=True)
            p = jnp.exp(s - m)
            l = jnp.sum(p, axis=1, keepdims=True)
            out.append(p * (1.0 / l))

        def o_gen(g, o, out):
            skip = min(max(WV - h0[g], 0), GS[g])
            if skip == GS[g]:
                out.append(None)
                return
            c0 = skip * DH // 128 * 128
            r0, nr = h0[g] * DH // 2 + c0 // 2, GS[g] * DH // 2 - c0 // 2
            on = max(1, ON * 8 // GS[g])
            ot = []
            n = 0
            while n < D // 128:
                nn = min(on, D // 128 - n)
                d = jnp.dot(gate(o[:, c0:]), _bf(wo_s[r0:r0 + nr, n * 128:(n + nn) * 128]), preferred_element_type=F32)
                ot.append(d)
                ZM.append(d[:, 0:128])
                n += nn
                yield nn * (nr * 2 // 128)
            out.append(jnp.concatenate(ot, axis=1))

        def pv_mxu(g, pn, out):
            r0 = h0[g] * DH // 2
            ot = []
            for u in range(GS[g] // 2):
                o = lax.dot_general(pn.astype(BF), _bf(v_s[sl, r0 + u * UR:r0 + (u + 1) * UR, :]),
                                    (((1,), (1,)), ((), ())), preferred_element_type=F32)
                ot.append(o)
                ZM.append(o[:, 0:128])
                yield 48
            out.append(jnp.where(gmask(g), jnp.concatenate(ot, axis=1), 0.0).astype(BF))

        vacc = [None] * (D // 128)

        def pv_gen(g, pn, out):
            tiles = [jnp.zeros((8, 128), F32) for _ in range(GS[g] * DH // 128)]
            for h in range(GS[g]):
                hh = h0[g] + h
                pb = jnp.broadcast_to(pn[h:h + 1, :], (8, W))
                pj0 = [pb[:, j * 128:(j + 1) * 128] for j in range(W // 128)]
                for i0 in range(0, DH // 16, VB):
                    z = tok()
                    if z is None:
                        pj = pj0
                    elif GATE == 5:
                        pbz = jnp.broadcast_to((pn + jnp.concatenate([z] * (W // 128), axis=1))[h:h + 1, :], (8, W))
                        pj = [pbz[:, j * 128:(j + 1) * 128] for j in range(W // 128)]
                    else:
                        pj = [p + z for p in pj0]
                    for i in range(i0, i0 + VB):
                        r0 = hh * (DH // 2) + i * 8
                        for j in range(W // 128):
                            if hh < NF:
                                lo = vf_s[0, r0:r0 + 8, j * 128:(j + 1) * 128] * pj[j]
                                hi = vf_s[1, r0:r0 + 8, j * 128:(j + 1) * 128] * pj[j]
                            else:
                                w = v_s[sl, r0:r0 + 8, j * 128:(j + 1) * 128]
                                lo = pltpu.bitcast(w << 16, F32) * pj[j]
                                hi = pltpu.bitcast(w & jnp.int32(-65536), F32) * pj[j]
                            if j == 0:
                                a_lo, a_hi = lo, hi
                            else:
                                a_lo, a_hi = a_lo + lo, a_hi + hi
                        rlo = jnp.sum(a_lo, axis=1, keepdims=True)
                        rhi = jnp.sum(a_hi, axis=1, keepdims=True)
                        if hh < WV:
                            for n in range(D // 128):
                                ww = wo_s[r0:r0 + 8, n * 128:(n + 1) * 128]
                                c = (pltpu.bitcast(ww << 16, F32) * rlo
                                     + pltpu.bitcast(ww & jnp.int32(-65536), F32) * rhi)
                                vacc[n] = c if vacc[n] is None else vacc[n] + c
                        else:
                            rg = h * DH + i * 16
                            t, off = rg // 128, rg % 128
                            tl = jnp.where(lidx == off, rlo, tiles[t])
                            tiles[t] = jnp.where(lidx == off + 1, rhi, tl)
                    ZV.append(a_hi)
                    yield VB
            out.append(jnp.concatenate(tiles, axis=1).astype(BF))
            if FWV and h0[g] < WV:
                PEND.append((g + FWV, vacc[0] + vacc[4]))

        PEND = []

        def interleave(ga, gb, na, nb):
            a = itertools.chain(*ga)
            done_a = not ga
            done_b = gb is None
            ia = ib = 0
            while not (done_a and done_b):
                if not done_a and (done_b or ia * nb <= ib * na):
                    try:
                        ia += next(a)
                    except StopIteration:
                        done_a = True
                else:
                    try:
                        ib += next(gb)
                    except StopIteration:
                        done_b = True

        acc = jnp.zeros((8, D), F32)
        ps, os_ = {}, {}
        for per in range(-1, ng + LAG):
            ga, na = [], 0
            o1, o2, o3, o4 = [], [], [], []
            for (pp, tk) in list(PEND):
                if pp == per:
                    FORCE.append(tk)
                    PEND[:] = [q for q in PEND if q[1] is not tk]
            if 0 <= per + 1 < ng:
                ga.append(q_gen(per + 1, o1))
                ga.append(s_gen(per + 1, o1, o2))
                na += 13 * (GS[per + 1] * DH // 128)
            gb = None
            if 0 <= per < ng:
                if per in MX:
                    ga.append(pv_mxu(per, ps.pop(per), o4))
                    na += 48 * GS[per] // 2
                else:
                    gb = pv_gen(per, ps.pop(per), o4)
            if 0 <= per - LAG < ng:
                ga.append(o_gen(per - LAG, os_.pop(per - LAG), o3))
                na += 5 * (GS[per - LAG] * DH // 128)
            interleave(ga, gb, max(na, 1), GS[min(max(per, 0), ng - 1)] * 12)
            if o2:
                ps[per + 1] = o2[0]
            if o3 and o3[0] is not None:
                acc = acc + o3[0]
            if o4:
                os_[per] = o4[0]
        if vacc[0] is not None:
            acc = acc + jnp.concatenate(vacc, axis=1)
        return jnp.broadcast_to(jnp.sum(acc, axis=0, keepdims=True), (8, D))

    def ffn(xn_f32):
        xn = xn_f32.astype(BF)
        r = jnp.sum(xn.astype(F32) * wr, axis=1, keepdims=True)
        gate = jnp.dot(xn, _bf(wg_s[...]), preferred_element_type=F32)
        up = jnp.dot(xn, _bf(wu_s[...]), preferred_element_type=F32)
        h = (gate * jax.nn.sigmoid(gate) * up).astype(BF)
        y = jnp.dot(h, _bf(wd_s[...]), preferred_element_type=F32)
        return xn.astype(F32) + y * jax.nn.sigmoid(r)

    def per_batch(b, out):
        @pl.when(b + 1 < B)
        def _():
            start_batch(b + 1)
        x = jnp.broadcast_to(
            jnp.sum(jnp.where(row4 == b, x_all, 0.0), axis=0, keepdims=True), (8, D))
        x = x + attention_stream(b, _layernorm(x).astype(BF))
        x = x + ffn(_layernorm(x))
        x = x + attention_resident(b, _layernorm(x).astype(BF))
        x = x + ffn(_layernorm(x))
        return jnp.where(row8 == b, x, out)

    out = lax.fori_loop(0, B, per_batch, jnp.zeros((8, D), F32))
    o_ref[...] = out[0:B].astype(BF)


@jax.jit
def pallas_interleave_layers__sliding_block_cached__moe_arch_mod__decode_kernel(
    A_x, A_k_cache, A_v_cache, A_wq, A_wo, B_x, B_w_r, B_w_gate, B_w_up, B_w_down,
):
    kT = jnp.swapaxes(A_k_cache, 2, 3).reshape(B * HD, SK)
    vT = jnp.swapaxes(A_v_cache, 2, 3).reshape(B * HD, SK)
    x2 = A_x.reshape(B, D)
    any_spec = pl.BlockSpec(memory_space=pl.ANY)
    out = pl.pallas_call(
        _kernel,
        out_shape=jax.ShapeDtypeStruct((B, D), BF),
        in_specs=[any_spec] * 9,
        out_specs=pl.BlockSpec(memory_space=pltpu.VMEM),
        scratch_shapes=[
            pltpu.VMEM((B, D), BF),
            pltpu.VMEM((D,), BF),
            pltpu.VMEM((NS, HD // 2, W), I32),
            pltpu.VMEM((NS, HD // 2, W), I32),
            pltpu.VMEM((2, max(NF, 1) * (DH // 2), W), F32),
            pltpu.VMEM((D // 2, HD), I32),
            pltpu.VMEM((HD // 2, D), I32),
            pltpu.VMEM((D // 2, F), I32),
            pltpu.VMEM((D // 2, F), I32),
            pltpu.VMEM((F // 2, D), I32),
            pltpu.SemaphoreType.DMA((7,)),
            pltpu.SemaphoreType.DMA((B, len(KC))),
            pltpu.SemaphoreType.DMA((B, len(VC))),
        ],
        compiler_params=pltpu.CompilerParams(vmem_limit_bytes=127 * 1024 * 1024),
    )(x2, kT, vT, A_wq, A_wo, B_w_r, B_w_gate, B_w_up, B_w_down)
    return out.reshape(B, 1, D)
```

```python
import itertools
import jax
import jax.numpy as jnp
import jax.experimental.pallas as pl
import jax.experimental.pallas.tpu as pltpu
from jax import lax

B, D = 4, 640
H, DH, SK = 32, 192, 4096
W = min(4096, max(256, SK // 4))
F = 1536
HD = H * DH
G = 8
NG = H // G
GW = G * DH
GR = GW // 2
UW = 2 * DH
UR = UW // 2
NU = H // 2
EPS = 1e-5
BF = jnp.bfloat16
F32 = jnp.float32
I32 = jnp.int32
SCALE = DH ** -0.5
SKEW = int(0)
VB = int(4)
QN = int(6)
SN = int(1)
ON = int(1)
LAG = int(2)
NS = int(2)
NF = int(30)
WV = int(6)
GATE = int(5)
SKM = int(-1)
FWV = int(0)
SORDER = 'x_wr_k_v_vf_wq_wo_wg_wu_wd_csg_csu_csq'.split('_')
FOLD = int(1)
FV = int(3)
KVN = int(2)
KVG = [int(c) for c in '0']
UB = int(32)
LN1P = int(1)
SPLIT = int(1)
ROLL = 0
def _chunks(s):
    c = [int(x) for x in s.split('_')]
    return list(zip(c[:-1], c[1:]))
KC = _chunks('0_8_16_24_32')
VC = _chunks('0_8_16_24_26_28_30_31_32')
DMA_ORDER = sorted([('k', i) for i in range(len(KC))] + [('v', i) for i in range(len(VC))],
                   key=lambda t: ((KC if t[0] == 'k' else VC)[t[1]][0] // G, t[0], t[1])) if int(1) else \
    [('k', i) for i in range(len(KC))] + [('v', i) for i in range(len(VC))]
GS = [int(c) for c in '48884']
assert sum(GS) == H
MX = [int(c) for c in '9']


def _layernorm(x):
    if LN1P:
        m = jnp.sum(x, axis=1, keepdims=True) * (1.0 / D)
        v = jnp.sum(x * x, axis=1, keepdims=True) * (1.0 / D) - m * m
        return (x - m) * lax.rsqrt(jnp.maximum(v, 0.0) + EPS)
    m = jnp.mean(x, axis=1, keepdims=True)
    d = x - m
    v = jnp.mean(d * d, axis=1, keepdims=True)
    return d / jnp.sqrt(v + EPS)


def _stats(x):
    m = jnp.sum(x, axis=1, keepdims=True) * (1.0 / D)
    v = jnp.sum(x * x, axis=1, keepdims=True) * (1.0 / D) - m * m
    return m, lax.rsqrt(jnp.maximum(v, 0.0) + EPS)


def _bf(x):
    return pltpu.bitcast(x, BF)


def _kernel(x_hbm, k_hbm, v_hbm, wq_hbm, wo_hbm, wr_hbm, wg_hbm, wu_hbm, wd_hbm,
            o_ref,
            *scr):
    sc = dict(zip(SORDER + ['sem_w', 'sem_k', 'sem_v'], scr))
    x_s, wr_s, k_s, v_s, vf_s, wq_s, wo_s, wg_s, wu_s, wd_s, sem_w, sem_k, sem_v = [sc[n] for n in ('x', 'wr', 'k', 'v', 'vf', 'wq', 'wo', 'wg', 'wu', 'wd', 'sem_w', 'sem_k', 'sem_v')]
    cs_g, cs_u, cs_q = sc['csg'], sc['csu'], sc['csq']
    k32 = k_hbm.bitcast(I32)
    v32 = v_hbm.bitcast(I32)

    def kv_copy(src32, dst, sems, b, ci, h0, h1):
        r0, nr = h0 * (DH // 2), (h1 - h0) * (DH // 2)
        g0 = b * (HD // 2) + r0
        if not isinstance(g0, int):
            g0 = pl.multiple_of(g0, DH // 2)
        return pltpu.make_async_copy(
            src32.at[pl.ds(g0, nr), pl.ds(SK - W, W)], dst.at[b % NS, pl.ds(r0, nr)], sems.at[b, ci])

    def k_copy(b, ci):
        return kv_copy(k32, k_s, sem_k, b, ci, *KC[ci])

    def v_copy(b, ci):
        return kv_copy(v32, v_s, sem_v, b, ci, *VC[ci])

    def start_batch(b):
        for kind, ci in DMA_ORDER:
            (k_copy if kind == "k" else v_copy)(b, ci).start()

    w_copies = [
        pltpu.make_async_copy(wq_hbm.bitcast(I32), wq_s, sem_w.at[0]),
        pltpu.make_async_copy(x_hbm, x_s, sem_w.at[1]),
        pltpu.make_async_copy(wr_hbm, wr_s, sem_w.at[2]),
        pltpu.make_async_copy(wo_hbm.bitcast(I32), wo_s, sem_w.at[3]),
        pltpu.make_async_copy(wg_hbm.bitcast(I32), wg_s, sem_w.at[4]),
        pltpu.make_async_copy(wu_hbm.bitcast(I32), wu_s, sem_w.at[5]),
        pltpu.make_async_copy(wd_hbm.bitcast(I32), wd_s, sem_w.at[6]),
    ]
    for c in w_copies:
        c.start()
    start_batch(0)

    row = lax.broadcasted_iota(I32, (8, GW), 0)
    col = lax.broadcasted_iota(I32, (8, GW), 1)
    mask = (col >= row * DH) & (col < row * DH + DH)
    r8 = lax.broadcasted_iota(I32, (8, 128), 0)
    c8 = lax.broadcasted_iota(I32, (8, 128), 1)
    lidx = c8 - 2 * r8
    row8 = lax.broadcasted_iota(I32, (8, D), 0)
    row4 = lax.broadcasted_iota(I32, (B, D), 0)

    for c in w_copies:
        c.wait()
    x_all = x_s[...].astype(F32)
    if FOLD:
        ones = jnp.ones((8, D), BF)
        cs_g[...] = jnp.dot(ones, _bf(wg_s[...]), preferred_element_type=F32)
        cs_u[...] = jnp.dot(ones, _bf(wu_s[...]), preferred_element_type=F32)
        for g in range(NG):
            cs_q[:, g * GW:(g + 1) * GW] = jnp.dot(ones, _bf(wq_s[:, g * GW:(g + 1) * GW]),
                                                   preferred_element_type=F32)
    wr = wr_s[...].reshape(1, D).astype(F32)

    def attention_stream(b, xn):
        sl = b % NS
        acc = jnp.zeros((8, D), F32)
        kw, vw = set(), set()

        def need(kind, h):
            chunks, done, cp = (KC, kw, k_copy) if kind == "k" else (VC, vw, v_copy)
            for ci, (h0, h1) in enumerate(chunks):
                if h0 <= h < h1 and ci not in done:
                    cp(b, ci).wait()
                    done.add(ci)

        def scores(g):
            q = jnp.dot(xn, _bf(wq_s[:, g * GW:(g + 1) * GW]), preferred_element_type=F32)
            qbd = jnp.where(mask, q, 0.0).astype(BF)
            need("k", g * G + G - 1)
            s = jnp.dot(qbd, _bf(k_s[sl, g * GR:(g + 1) * GR, :]), preferred_element_type=F32) * SCALE
            m = jnp.max(s, axis=1, keepdims=True)
            p = jnp.exp(s - m)
            l = jnp.sum(p, axis=1, keepdims=True)
            return (p * (1.0 / l)).astype(BF)

        pns = {}
        for g in range(NG):
            if g not in pns:
                ci = [i for i, (h0, h1) in enumerate(KC) if h0 <= g * G < h1][0]
                for g2 in range(g, NG):
                    if KC[ci][0] <= g2 * G < KC[ci][1]:
                        pns[g2] = scores(g2)
            pn = pns.pop(g)
            h = g * G
            while h < (g + 1) * G:
                ci = [i for i, (h0, h1) in enumerate(VC) if h0 <= h < h1][0]
                nh = min(2, VC[ci][1] - h)
                need("v", h)
                r0, nr = h * (DH // 2), nh * (DH // 2)
                o = lax.dot_general(pn, _bf(v_s[sl, r0:r0 + nr, :]), (((1,), (1,)), ((), ())),
                                    preferred_element_type=F32)
                c0 = (h - g * G) * DH
                if nh == 2:
                    msk = mask[:, c0:c0 + nh * DH]
                else:
                    msk = lax.broadcasted_iota(I32, (8, DH), 0) == (h - g * G)
                o = jnp.where(msk, o, 0.0).astype(BF)
                acc = acc + jnp.dot(o, _bf(wo_s[r0:r0 + nr, :]), preferred_element_type=F32)
                h += nh
                if h == VC[ci][1] and VC[ci][0] < NF:
                    u0, u1 = VC[ci][0] * (DH // 2) // UB, min(VC[ci][1], NF) * (DH // 2) // UB

                    def widen(i, c):
                        r = pl.multiple_of(i * UB, UB)
                        w = v_s[sl, pl.ds(r, UB), :]
                        vf_s[0, pl.ds(r, UB), :] = pltpu.bitcast(w << 16, F32)
                        vf_s[1, pl.ds(r, UB), :] = pltpu.bitcast(w & jnp.int32(-65536), F32)
                        return c
                    lax.fori_loop(u0, u1, widen, 0)
        return jnp.broadcast_to(jnp.sum(acc, axis=0, keepdims=True), (8, D))

    def attention_resident(b, xn, cq=None, invq=None):
        sl = b % NS
        ZM = []
        ng = len(GS)
        h0 = [sum(GS[:i]) for i in range(ng)]

        def tok():
            return ZM[-1 - SKEW] * 0.0 if (SKEW >= 0 and len(ZM) > SKEW) else None

        ZV = []

        FORCE = []

        def gate(lhs):
            if FORCE:
                z = FORCE.pop() * 0.0
                return (lhs.astype(F32) + jnp.concatenate([z] * (lhs.shape[1] // 128), axis=1)).astype(BF)
            if SKM < 0 or len(ZV) <= SKM:
                return lhs
            z = ZV[-1 - SKM] * 0.0
            return (lhs.astype(F32) + jnp.concatenate([z] * (lhs.shape[1] // 128), axis=1)).astype(BF)

        def gmask(g):
            n = GS[g] * DH
            row = lax.broadcasted_iota(I32, (8, n), 0)
            col = lax.broadcasted_iota(I32, (8, n), 1)
            return (col >= row * DH) & (col < row * DH + DH)

        def q_gen(g, out):
            nt = GS[g] * DH // 128
            c0 = h0[g] * DH
            qt = []
            t = 0
            while t < nt:
                n = min(QN, nt - t)
                d = jnp.dot(gate(xn), _bf(wq_s[:, c0 + t * 128:c0 + (t + n) * 128]), preferred_element_type=F32)
                ZM.append(d[:, 0:128])
                if cq is not None:
                    d = (d - cq * cs_q[:, c0 + t * 128:c0 + (t + n) * 128]) * invq
                qt.append(d)
                t += n
                yield n * 5
            qf = jnp.concatenate(qt, axis=1)
            out.append(jnp.where(gmask(g), qf, 0.0).astype(BF))
            out.append(qf.astype(BF).astype(F32))

        def s_gen(g, qsrc, out):
            kv = KVN if g in KVG else 0
            nm = GS[g] - kv
            r0, nr = h0[g] * DH // 2, nm * DH // 2
            sn = max(1, SN * 8 // max(nm, 1))
            st = []
            qcols = {}
            row8_ = lax.broadcasted_iota(I32, (8, 128), 0)
            for j in range(0, W // 128, sn):
                d = jnp.dot(gate(qsrc[0][:, 0:nm * DH]), _bf(k_s[sl, r0:r0 + nr, j * 128:(j + sn) * 128]),
                            preferred_element_type=F32)
                ZM.append(d[:, 0:128])
                if kv:
                    if not qcols:
                        for h in range(nm, GS[g]):
                            for i in range(DH // 16):
                                rg = h * DH + i * 16
                                t, off = rg // 128, rg % 128
                                qt_ = qsrc[1][:, t * 128:(t + 1) * 128]
                                qcols[h, i] = (jnp.sum(jnp.where(lidx == off, qt_, 0.0), axis=1, keepdims=True),
                                               jnp.sum(jnp.where(lidx == off + 1, qt_, 0.0), axis=1, keepdims=True))
                    add = []
                    for jj in range(j, j + sn):
                        tot = None
                        for h in range(nm, GS[g]):
                            a = None
                            for i in range(DH // 16):
                                rr = (h0[g] + h) * (DH // 2) + i * 8
                                w = k_s[sl, rr:rr + 8, jj * 128:(jj + 1) * 128]
                                c2 = (pltpu.bitcast(w << 16, F32) * qcols[h, i][0]
                                      + pltpu.bitcast(w & jnp.int32(-65536), F32) * qcols[h, i][1])
                                a = c2 if a is None else a + c2
                            a = jnp.broadcast_to(jnp.sum(a, axis=0, keepdims=True), (8, 128))
                            a = jnp.where(row8_ == h, a, 0.0)
                            tot = a if tot is None else tot + a
                        add.append(tot)
                    d = d + jnp.concatenate(add, axis=1)
                st.append(d)
                yield sn * (nm * DH // 128)
            s = jnp.concatenate(st, axis=1) * SCALE
            m = jnp.max(s, axis=1, keepdims=True)
            p = jnp.exp(s - m)
            l = jnp.sum(p, axis=1, keepdims=True)
            out.append(p * (1.0 / l))

        def o_gen(g, o, out):
            skip = min(max(WV - h0[g], 0), GS[g])
            if skip == GS[g]:
                out.append(None)
                return
            c0 = skip * DH // 128 * 128
            r0, nr = h0[g] * DH // 2 + c0 // 2, GS[g] * DH // 2 - c0 // 2
            on = max(1, ON * 8 // GS[g])
            ot = []
            n = 0
            while n < D // 128:
                nn = min(on, D // 128 - n)
                d = jnp.dot(gate(o[:, c0:]), _bf(wo_s[r0:r0 + nr, n * 128:(n + nn) * 128]), preferred_element_type=F32)
                ot.append(d)
                ZM.append(d[:, 0:128])
                n += nn
                yield nn * (nr * 2 // 128)
            out.append(jnp.concatenate(ot, axis=1))

        def pv_mxu(g, pn, out):
            r0 = h0[g] * DH // 2
            ot = []
            for u in range(GS[g] // 2):
                o = lax.dot_general(pn.astype(BF), _bf(v_s[sl, r0 + u * UR:r0 + (u + 1) * UR, :]),
                                    (((1,), (1,)), ((), ())), preferred_element_type=F32)
                ot.append(o)
                ZM.append(o[:, 0:128])
                yield 48
            out.append(jnp.where(gmask(g), jnp.concatenate(ot, axis=1), 0.0).astype(BF))

        vacc = [None] * (D // 128)

        def pv_gen(g, pn, out):
            tiles = [jnp.zeros((8, 128), F32) for _ in range(GS[g] * DH // 128)]
            for h in range(GS[g]):
                hh = h0[g] + h
                pb = jnp.broadcast_to(pn[h:h + 1, :], (8, W))
                pj0 = [pb[:, j * 128:(j + 1) * 128] for j in range(W // 128)]
                for i0 in range(0, DH // 16, VB):
                    z = tok()
                    if z is None:
                        pj = pj0
                    elif GATE == 5:
                        pbz = jnp.broadcast_to((pn + jnp.concatenate([z] * (W // 128), axis=1))[h:h + 1, :], (8, W))
                        pj = [pbz[:, j * 128:(j + 1) * 128] for j in range(W // 128)]
                    else:
                        pj = [p + z for p in pj0]
                    for i in range(i0, i0 + VB):
                        r0 = hh * (DH // 2) + i * 8
                        for j in range(W // 128):
                            if hh < NF:
                                lo = vf_s[0, r0:r0 + 8, j * 128:(j + 1) * 128] * pj[j]
                                hi = vf_s[1, r0:r0 + 8, j * 128:(j + 1) * 128] * pj[j]
                            else:
                                w = v_s[sl, r0:r0 + 8, j * 128:(j + 1) * 128]
                                lo = pltpu.bitcast(w << 16, F32) * pj[j]
                                hi = pltpu.bitcast(w & jnp.int32(-65536), F32) * pj[j]
                            if j == 0:
                                a_lo, a_hi = lo, hi
                            else:
                                a_lo, a_hi = a_lo + lo, a_hi + hi
                        rlo = jnp.sum(a_lo, axis=1, keepdims=True)
                        rhi = jnp.sum(a_hi, axis=1, keepdims=True)
                        if hh < WV:
                            for n in range(D // 128):
                                ww = wo_s[r0:r0 + 8, n * 128:(n + 1) * 128]
                                c = (pltpu.bitcast(ww << 16, F32) * rlo
                                     + pltpu.bitcast(ww & jnp.int32(-65536), F32) * rhi)
                                vacc[n] = c if vacc[n] is None else vacc[n] + c
                        else:
                            rg = h * DH + i * 16
                            t, off = rg // 128, rg % 128
                            tl = jnp.where(lidx == off, rlo, tiles[t])
                            tiles[t] = jnp.where(lidx == off + 1, rhi, tl)
                    ZV.append(a_hi)
                    yield VB
            out.append(jnp.concatenate(tiles, axis=1).astype(BF))
            if FWV and h0[g] < WV:
                PEND.append((g + FWV, vacc[0] + vacc[4]))

        PEND = []

        def interleave(ga, gb, na, nb):
            a = itertools.chain(*ga)
            done_a = not ga
            done_b = gb is None
            ia = ib = 0
            while not (done_a and done_b):
                if not done_a and (done_b or ia * nb <= ib * na):
                    try:
                        ia += next(a)
                    except StopIteration:
                        done_a = True
                else:
                    try:
                        ib += next(gb)
                    except StopIteration:
                        done_b = True

        acc = jnp.zeros((8, D), F32)
        ps, os_ = {}, {}
        for per in range(-1, ng + LAG):
            ga, na = [], 0
            o1, o2, o3, o4 = [], [], [], []
            for (pp, tk) in list(PEND):
                if pp == per:
                    FORCE.append(tk)
                    PEND[:] = [q for q in PEND if q[1] is not tk]
            if 0 <= per + 1 < ng:
                ga.append(q_gen(per + 1, o1))
                ga.append(s_gen(per + 1, o1, o2))
                na += 13 * (GS[per + 1] * DH // 128)
            gb = None
            if 0 <= per < ng:
                if per in MX:
                    ga.append(pv_mxu(per, ps.pop(per), o4))
                    na += 48 * GS[per] // 2
                else:
                    gb = pv_gen(per, ps.pop(per), o4)
            if 0 <= per - LAG < ng:
                ga.append(o_gen(per - LAG, os_.pop(per - LAG), o3))
                na += 5 * (GS[per - LAG] * DH // 128)
            interleave(ga, gb, max(na, 1), GS[min(max(per, 0), ng - 1)] * 12)
            if o2:
                ps[per + 1] = o2[0]
            if o3 and o3[0] is not None:
                acc = acc + o3[0]
            if o4:
                os_[per] = o4[0]
        if vacc[0] is not None:
            acc = acc + jnp.concatenate(vacc, axis=1)
        return jnp.broadcast_to(jnp.sum(acc, axis=0, keepdims=True), (8, D))

    def ffn(xn_f32):
        xn = xn_f32.astype(BF)
        r = jnp.sum(xn.astype(F32) * wr, axis=1, keepdims=True)
        gate = jnp.dot(xn, _bf(wg_s[...]), preferred_element_type=F32)
        up = jnp.dot(xn, _bf(wu_s[...]), preferred_element_type=F32)
        h = (gate * jax.nn.sigmoid(gate) * up).astype(BF)
        y = jnp.dot(h, _bf(wd_s[...]), preferred_element_type=F32)
        return xn.astype(F32) + y * jax.nn.sigmoid(r)

    def ffn_fold(x, m_prev):
        u = (x - m_prev).astype(BF)
        m, inv = _stats(x)
        c = m - m_prev
        xn = ((x - m) * inv).astype(BF).astype(F32)
        r = jnp.sum(xn * wr, axis=1, keepdims=True)
        if FV:
            uf = u.astype(F32)
            cols = []
            for i in range(D // 16):
                t, off = (i * 16) // 128, (i * 16) % 128
                ut = uf[:, t * 128:(t + 1) * 128]
                cols.append((jnp.sum(jnp.where(lidx == off, ut, 0.0), axis=1, keepdims=True),
                             jnp.sum(jnp.where(lidx == off + 1, ut, 0.0), axis=1, keepdims=True)))

            def proj(w_s):
                nm = F - FV * 128
                parts = [jnp.dot(u, _bf(w_s[:, 0:nm]), preferred_element_type=F32)]
                for n in range(nm // 128, F // 128):
                    a = None
                    for i in range(D // 16):
                        w = w_s[i * 8:(i + 1) * 8, n * 128:(n + 1) * 128]
                        c2 = (pltpu.bitcast(w << 16, F32) * cols[i][0]
                              + pltpu.bitcast(w & jnp.int32(-65536), F32) * cols[i][1])
                        a = c2 if a is None else a + c2
                    parts.append(jnp.broadcast_to(jnp.sum(a, axis=0, keepdims=True), (8, 128)))
                return jnp.concatenate(parts, axis=1)
            gate = (proj(wg_s) - c * cs_g[...]) * inv
            up = (proj(wu_s) - c * cs_u[...]) * inv
        else:
            gate = (jnp.dot(u, _bf(wg_s[...]), preferred_element_type=F32) - c * cs_g[...]) * inv
            up = (jnp.dot(u, _bf(wu_s[...]), preferred_element_type=F32) - c * cs_u[...]) * inv
        h = (gate * jax.nn.sigmoid(gate) * up).astype(BF)
        y = jnp.dot(h, _bf(wd_s[...]), preferred_element_type=F32)
        return x + xn + y * jax.nn.sigmoid(r), m

    def per_batch(b, out):
        @pl.when(b + 1 < B)
        def _():
            start_batch(b + 1)
        x = jnp.broadcast_to(
            jnp.sum(jnp.where(row4 == b, x_all, 0.0), axis=0, keepdims=True), (8, D))
        if FOLD:
            m0, inv0 = _stats(x)
            x = x + attention_stream(b, ((x - m0) * inv0).astype(BF))
            x, m1 = ffn_fold(x, m0)
            m2, inv2 = _stats(x)
            x = x + attention_resident(b, (x - m1).astype(BF), m2 - m1, inv2)
            x, _ = ffn_fold(x, m2)
        else:
            x = x + attention_stream(b, _layernorm(x).astype(BF))
            x = x + ffn(_layernorm(x))
            x = x + attention_resident(b, _layernorm(x).astype(BF))
            x = x + ffn(_layernorm(x))
        return jnp.where(row8 == b, x, out)

    out = lax.fori_loop(0, B, per_batch, jnp.zeros((8, D), F32))
    o_ref[...] = out[0:B].astype(BF)


@jax.jit
def pallas_interleave_layers__sliding_block_cached__moe_arch_mod__decode_kernel(
    A_x, A_k_cache, A_v_cache, A_wq, A_wo, B_x, B_w_r, B_w_gate, B_w_up, B_w_down,
):
    SHAPES = dict(
        x=pltpu.VMEM((B, D), BF), wr=pltpu.VMEM((D,), BF),
        k=pltpu.VMEM((NS, HD // 2, W), I32), v=pltpu.VMEM((NS, HD // 2, W), I32),
        vf=pltpu.VMEM((2, max(NF, 1) * (DH // 2), W), F32),
        wq=pltpu.VMEM((D // 2, HD), I32), wo=pltpu.VMEM((HD // 2, D), I32),
        wg=pltpu.VMEM((D // 2, F), I32), wu=pltpu.VMEM((D // 2, F), I32), wd=pltpu.VMEM((F // 2, D), I32),
        csg=pltpu.VMEM((8, F), F32), csu=pltpu.VMEM((8, F), F32), csq=pltpu.VMEM((8, HD), F32))
    kT = jnp.swapaxes(A_k_cache, 2, 3).reshape(B * HD, SK)
    vT = jnp.swapaxes(A_v_cache, 2, 3).reshape(B * HD, SK)
    x2 = A_x.reshape(B, D)
    any_spec = pl.BlockSpec(memory_space=pl.ANY)
    out = pl.pallas_call(
        _kernel,
        out_shape=jax.ShapeDtypeStruct((B, D), BF),
        in_specs=[any_spec] * 9,
        out_specs=pl.BlockSpec(memory_space=pltpu.VMEM),
        scratch_shapes=[SHAPES[n] for n in SORDER] + [
            pltpu.SemaphoreType.DMA((7,)),
            pltpu.SemaphoreType.DMA((B, len(KC))),
            pltpu.SemaphoreType.DMA((B, len(VC))),
        ],
        compiler_params=pltpu.CompilerParams(vmem_limit_bytes=127 * 1024 * 1024),
    )(x2, kT, vT, A_wq, A_wo, B_w_r, B_w_gate, B_w_up, B_w_down)
    return out.reshape(B, 1, D)
```

```python
import itertools

import jax
import jax.numpy as jnp
import jax.experimental.pallas as pl
import jax.experimental.pallas.tpu as pltpu
from jax import lax

B, D = 4, 640
H, DH, SK = 32, 192, 4096
W = min(4096, max(256, SK // 4))
F = 1536
HD = H * DH
HR = DH // 2
G = 8
GW = G * DH
EPS = 1e-5
SCALE = DH ** -0.5
BF, F32, I32 = jnp.bfloat16, jnp.float32, jnp.int32
HI_MASK = -65536

NSLOT = 2
K_CHUNKS = [(0, 8), (8, 16), (16, 24), (24, 32)]
V_CHUNKS = [(0, 8), (8, 16), (16, 24), (24, 26), (26, 28), (28, 30), (30, 31), (31, 32)]
DMA_ORDER = sorted([("k", i) for i in range(len(K_CHUNKS))] + [("v", i) for i in range(len(V_CHUNKS))],
                   key=lambda t: ((K_CHUNKS if t[0] == "k" else V_CHUNKS)[t[1]][0] // G, t[0], t[1]))

GROUPS = [4, 8, 8, 8, 4]
N_F32 = 30
WO_VPU = 7
QK_VPU = 2
FFN_VPU = 2
LAG = 2
QN, VB, UB = 12, 4, 32
assert sum(GROUPS) == H


def _bf(x):
    return pltpu.bitcast(x, BF)


def _lo(w):
    return pltpu.bitcast(w << 16, F32)


def _hi(w):
    return pltpu.bitcast(w & jnp.int32(HI_MASK), F32)


def _stats(x):
    m = jnp.sum(x, axis=1, keepdims=True) * (1.0 / D)
    v = jnp.sum(x * x, axis=1, keepdims=True) * (1.0 / D) - m * m
    return m, lax.rsqrt(jnp.maximum(v, 0.0) + EPS)


def _softmax(s):
    m = jnp.max(s, axis=1, keepdims=True)
    p = jnp.exp(s - m)
    l = jnp.sum(p, axis=1, keepdims=True)
    return p * (1.0 / l)


def _block_mask(nh):
    row = lax.broadcasted_iota(I32, (8, nh * DH), 0)
    col = lax.broadcasted_iota(I32, (8, nh * DH), 1)
    return (col >= row * DH) & (col < row * DH + DH)


def _kernel(x_hbm, k_hbm, v_hbm, wq_hbm, wo_hbm, wr_hbm, wg_hbm, wu_hbm, wd_hbm,
            o_ref,
            x_s, wr_s, k_s, v_s, vf_s, wq_s, wo_s, wg_s, wu_s, wd_s, cs_g, cs_u, cs_q,
            sem_w, sem_k, sem_v):
    k32 = k_hbm.bitcast(I32)
    v32 = v_hbm.bitcast(I32)

    def kv_copy(src, dst, sems, b, ci, h0, h1):
        r0, nr = h0 * HR, (h1 - h0) * HR
        g0 = b * (HD // 2) + r0
        if not isinstance(g0, int):
            g0 = pl.multiple_of(g0, HR)
        return pltpu.make_async_copy(
            src.at[pl.ds(g0, nr), pl.ds(SK - W, W)], dst.at[b % NSLOT, pl.ds(r0, nr)], sems.at[b, ci])

    def k_copy(b, ci):
        return kv_copy(k32, k_s, sem_k, b, ci, *K_CHUNKS[ci])

    def v_copy(b, ci):
        return kv_copy(v32, v_s, sem_v, b, ci, *V_CHUNKS[ci])

    def start_batch(b):
        for kind, ci in DMA_ORDER:
            (k_copy if kind == "k" else v_copy)(b, ci).start()

    w_copies = [
        pltpu.make_async_copy(wq_hbm.bitcast(I32), wq_s, sem_w.at[0]),
        pltpu.make_async_copy(x_hbm, x_s, sem_w.at[1]),
        pltpu.make_async_copy(wr_hbm, wr_s, sem_w.at[2]),
        pltpu.make_async_copy(wo_hbm.bitcast(I32), wo_s, sem_w.at[3]),
        pltpu.make_async_copy(wg_hbm.bitcast(I32), wg_s, sem_w.at[4]),
        pltpu.make_async_copy(wu_hbm.bitcast(I32), wu_s, sem_w.at[5]),
        pltpu.make_async_copy(wd_hbm.bitcast(I32), wd_s, sem_w.at[6]),
    ]
    for c in w_copies:
        c.start()
    start_batch(0)

    mask = _block_mask(G)
    lidx = lax.broadcasted_iota(I32, (8, 128), 1) - 2 * lax.broadcasted_iota(I32, (8, 128), 0)
    row8 = lax.broadcasted_iota(I32, (8, D), 0)
    row4 = lax.broadcasted_iota(I32, (B, D), 0)

    for c in w_copies:
        c.wait()
    x_all = x_s[...].astype(F32)
    wr = wr_s[...].reshape(1, D).astype(F32)
    ones = jnp.ones((8, D), BF)
    cs_g[...] = jnp.dot(ones, _bf(wg_s[...]), preferred_element_type=F32)
    cs_u[...] = jnp.dot(ones, _bf(wu_s[...]), preferred_element_type=F32)
    for g in range(H // G):
        cs_q[:, g * GW:(g + 1) * GW] = jnp.dot(ones, _bf(wq_s[:, g * GW:(g + 1) * GW]),
                                               preferred_element_type=F32)

    def columns(row_f32, n16):
        cols = []
        for i in range(n16):
            t, off = (i * 16) // 128, (i * 16) % 128
            tile = row_f32[:, t * 128:(t + 1) * 128]
            cols.append((jnp.sum(jnp.where(lidx == off, tile, 0.0), axis=1, keepdims=True),
                         jnp.sum(jnp.where(lidx == off + 1, tile, 0.0), axis=1, keepdims=True)))
        return cols

    def attention_stream(b, xn):
        sl = b % NSLOT
        acc = jnp.zeros((8, D), F32)
        k_done, v_done = set(), set()

        def need(chunks, done, copy, h):
            for ci, (h0, h1) in enumerate(chunks):
                if h0 <= h < h1 and ci not in done:
                    copy(b, ci).wait()
                    done.add(ci)

        for g in range(H // G):
            q = jnp.dot(xn, _bf(wq_s[:, g * GW:(g + 1) * GW]), preferred_element_type=F32)
            qbd = jnp.where(mask, q, 0.0).astype(BF)
            need(K_CHUNKS, k_done, k_copy, g * G + G - 1)
            s = jnp.dot(qbd, _bf(k_s[sl, g * G * HR:(g + 1) * G * HR, :]), preferred_element_type=F32)
            pn = _softmax(s * SCALE).astype(BF)
            h = g * G
            while h < (g + 1) * G:
                ci = [i for i, (h0, h1) in enumerate(V_CHUNKS) if h0 <= h < h1][0]
                nh = min(2, V_CHUNKS[ci][1] - h)
                need(V_CHUNKS, v_done, v_copy, h)
                r0, nr = h * HR, nh * HR
                o = lax.dot_general(pn, _bf(v_s[sl, r0:r0 + nr, :]), (((1,), (1,)), ((), ())),
                                    preferred_element_type=F32)
                c0 = (h - g * G) * DH
                if nh == 2:
                    msk = mask[:, c0:c0 + nh * DH]
                else:
                    msk = lax.broadcasted_iota(I32, (8, DH), 0) == (h - g * G)
                o = jnp.where(msk, o, 0.0).astype(BF)
                acc = acc + jnp.dot(o, _bf(wo_s[r0:r0 + nr, :]), preferred_element_type=F32)
                h += nh
                if h == V_CHUNKS[ci][1] and V_CHUNKS[ci][0] < N_F32:
                    u0, u1 = V_CHUNKS[ci][0] * HR // UB, min(V_CHUNKS[ci][1], N_F32) * HR // UB

                    def widen(i, c):
                        r = pl.multiple_of(i * UB, UB)
                        w = v_s[sl, pl.ds(r, UB), :]
                        vf_s[0, pl.ds(r, UB), :] = _lo(w)
                        vf_s[1, pl.ds(r, UB), :] = _hi(w)
                        return c
                    lax.fori_loop(u0, u1, widen, 0)
        return jnp.broadcast_to(jnp.sum(acc, axis=0, keepdims=True), (8, D))

    def attention_resident(b, u, cq, inv):
        sl = b % NSLOT
        ng = len(GROUPS)
        h0 = [sum(GROUPS[:i]) for i in range(ng)]
        mxu_results = []
        vacc = [None] * (D // 128)

        def q_gen(g, out):
            nt = GROUPS[g] * DH // 128
            c0 = h0[g] * DH
            qt, t = [], 0
            while t < nt:
                n = min(QN, nt - t)
                cols = slice(c0 + t * 128, c0 + (t + n) * 128)
                d = jnp.dot(u, _bf(wq_s[:, cols]), preferred_element_type=F32)
                mxu_results.append(d[:, 0:128])
                qt.append((d - cq * cs_q[:, cols]) * inv)
                t += n
                yield n * 5
            q = jnp.concatenate(qt, axis=1)
            out.append(jnp.where(_block_mask(GROUPS[g]), q, 0.0).astype(BF))
            out.append(q.astype(BF).astype(F32))

        def s_gen(g, qs, out):
            nv = QK_VPU if g == 0 else 0
            nm = GROUPS[g] - nv
            r0, nr = h0[g] * HR, nm * HR
            sn = max(1, 8 // nm)
            st, qcols = [], {}
            sub = lax.broadcasted_iota(I32, (8, 128), 0)
            for j in range(0, W // 128, sn):
                d = jnp.dot(qs[0][:, 0:nm * DH], _bf(k_s[sl, r0:r0 + nr, j * 128:(j + sn) * 128]),
                            preferred_element_type=F32)
                mxu_results.append(d[:, 0:128])
                if nv:
                    if not qcols:
                        allc = columns(qs[1], GROUPS[g] * DH // 16)
                        for h in range(nm, GROUPS[g]):
                            for i in range(DH // 16):
                                qcols[h, i] = allc[h * (DH // 16) + i]
                    add = []
                    for jj in range(j, j + sn):
                        tot = None
                        for h in range(nm, GROUPS[g]):
                            a = None
                            for i in range(DH // 16):
                                rr = (h0[g] + h) * HR + i * 8
                                w = k_s[sl, rr:rr + 8, jj * 128:(jj + 1) * 128]
                                c2 = _lo(w) * qcols[h, i][0] + _hi(w) * qcols[h, i][1]
                                a = c2 if a is None else a + c2
                            a = jnp.broadcast_to(jnp.sum(a, axis=0, keepdims=True), (8, 128))
                            a = jnp.where(sub == h, a, 0.0)
                            tot = a if tot is None else tot + a
                        add.append(tot)
                    d = d + jnp.concatenate(add, axis=1)
                st.append(d)
                yield sn * (nm * DH // 128)
            out.append(_softmax(jnp.concatenate(st, axis=1) * SCALE))

        def o_gen(g, o, out):
            skip = min(max(WO_VPU - h0[g], 0), GROUPS[g])
            if skip == GROUPS[g]:
                out.append(None)
                return
            c0 = skip * DH // 128 * 128
            r0, nr = h0[g] * HR + c0 // 2, GROUPS[g] * HR - c0 // 2
            on = max(1, 8 // GROUPS[g])
            ot, n = [], 0
            while n < D // 128:
                nn = min(on, D // 128 - n)
                d = jnp.dot(o[:, c0:], _bf(wo_s[r0:r0 + nr, n * 128:(n + nn) * 128]),
                            preferred_element_type=F32)
                ot.append(d)
                mxu_results.append(d[:, 0:128])
                n += nn
                yield nn * (nr * 2 // 128)
            out.append(jnp.concatenate(ot, axis=1))

        def pv_gen(g, pn, out):
            tiles = [jnp.zeros((8, 128), F32) for _ in range(GROUPS[g] * DH // 128)]
            for h in range(GROUPS[g]):
                hh = h0[g] + h
                for i0 in range(0, DH // 16, VB):
                    z = mxu_results[-1] * 0.0
                    pb = jnp.broadcast_to((pn + jnp.concatenate([z] * (W // 128), axis=1))[h:h + 1, :], (8, W))
                    pj = [pb[:, j * 128:(j + 1) * 128] for j in range(W // 128)]
                    for i in range(i0, i0 + VB):
                        r0 = hh * HR + i * 8
                        for j in range(W // 128):
                            if hh < N_F32:
                                lo = vf_s[0, r0:r0 + 8, j * 128:(j + 1) * 128] * pj[j]
                                hi = vf_s[1, r0:r0 + 8, j * 128:(j + 1) * 128] * pj[j]
                            else:
                                w = v_s[sl, r0:r0 + 8, j * 128:(j + 1) * 128]
                                lo, hi = _lo(w) * pj[j], _hi(w) * pj[j]
                            a_lo, a_hi = (lo, hi) if j == 0 else (a_lo + lo, a_hi + hi)
                        rlo = jnp.sum(a_lo, axis=1, keepdims=True)
                        rhi = jnp.sum(a_hi, axis=1, keepdims=True)
                        if hh < WO_VPU:
                            for n in range(D // 128):
                                ww = wo_s[r0:r0 + 8, n * 128:(n + 1) * 128]
                                c = _lo(ww) * rlo + _hi(ww) * rhi
                                vacc[n] = c if vacc[n] is None else vacc[n] + c
                        else:
                            rg = h * DH + i * 16
                            t, off = rg // 128, rg % 128
                            tl = jnp.where(lidx == off, rlo, tiles[t])
                            tiles[t] = jnp.where(lidx == off + 1, rhi, tl)
                    yield VB
            out.append(jnp.concatenate(tiles, axis=1).astype(BF))

        def interleave(mxu_gens, vpu_gen, na, nb):
            a = itertools.chain(*mxu_gens)
            done_a, done_b = not mxu_gens, vpu_gen is None
            ia = ib = 0
            while not (done_a and done_b):
                if not done_a and (done_b or ia * nb <= ib * na):
                    try:
                        ia += next(a)
                    except StopIteration:
                        done_a = True
                else:
                    try:
                        ib += next(vpu_gen)
                    except StopIteration:
                        done_b = True

        acc = jnp.zeros((8, D), F32)
        ps, os_ = {}, {}
        for per in range(-1, ng + LAG):
            gens, na = [], 0
            o1, o2, o3, o4 = [], [], [], []
            if 0 <= per + 1 < ng:
                gens += [q_gen(per + 1, o1), s_gen(per + 1, o1, o2)]
                na += 13 * (GROUPS[per + 1] * DH // 128)
            vpu = pv_gen(per, ps.pop(per), o4) if 0 <= per < ng else None
            if 0 <= per - LAG < ng:
                gens.append(o_gen(per - LAG, os_.pop(per - LAG), o3))
                na += 5 * (GROUPS[per - LAG] * DH // 128)
            interleave(gens, vpu, max(na, 1), GROUPS[min(max(per, 0), ng - 1)] * 12)
            if o2:
                ps[per + 1] = o2[0]
            if o3 and o3[0] is not None:
                acc = acc + o3[0]
            if o4:
                os_[per] = o4[0]
        if vacc[0] is not None:
            acc = acc + jnp.concatenate(vacc, axis=1)
        return jnp.broadcast_to(jnp.sum(acc, axis=0, keepdims=True), (8, D))

    def ffn(x, m_prev):
        u = (x - m_prev).astype(BF)
        m, inv = _stats(x)
        c = m - m_prev
        xn = ((x - m) * inv).astype(BF).astype(F32)
        r = jnp.sum(xn * wr, axis=1, keepdims=True)
        cols = columns(u.astype(F32), D // 16)

        def proj(w_s):
            nm = F - FFN_VPU * 128
            parts = [jnp.dot(u, _bf(w_s[:, 0:nm]), preferred_element_type=F32)]
            for n in range(nm // 128, F // 128):
                a = None
                for i in range(D // 16):
                    w = w_s[i * 8:(i + 1) * 8, n * 128:(n + 1) * 128]
                    c2 = _lo(w) * cols[i][0] + _hi(w) * cols[i][1]
                    a = c2 if a is None else a + c2
                parts.append(jnp.broadcast_to(jnp.sum(a, axis=0, keepdims=True), (8, 128)))
            return jnp.concatenate(parts, axis=1)

        gate = (proj(wg_s) - c * cs_g[...]) * inv
        up = (proj(wu_s) - c * cs_u[...]) * inv
        h = (gate * jax.nn.sigmoid(gate) * up).astype(BF)
        y = jnp.dot(h, _bf(wd_s[...]), preferred_element_type=F32)
        return x + xn + y * jax.nn.sigmoid(r), m

    def per_batch(b, out):
        @pl.when(b + 1 < B)
        def _():
            start_batch(b + 1)

        x = jnp.broadcast_to(jnp.sum(jnp.where(row4 == b, x_all, 0.0), axis=0, keepdims=True), (8, D))
        m0, inv0 = _stats(x)
        x = x + attention_stream(b, ((x - m0) * inv0).astype(BF))
        x, m1 = ffn(x, m0)
        m2, inv2 = _stats(x)
        x = x + attention_resident(b, (x - m1).astype(BF), m2 - m1, inv2)
        x, _ = ffn(x, m2)
        return jnp.where(row8 == b, x, out)

    out = lax.fori_loop(0, B, per_batch, jnp.zeros((8, D), F32))
    o_ref[...] = out[0:B].astype(BF)


@jax.jit
def pallas_interleave_layers__sliding_block_cached__moe_arch_mod__decode_kernel(
    A_x: jax.Array,
    A_k_cache: jax.Array,
    A_v_cache: jax.Array,
    A_wq: jax.Array,
    A_wo: jax.Array,
    B_x: jax.Array,
    B_w_r: jax.Array,
    B_w_gate: jax.Array,
    B_w_up: jax.Array,
    B_w_down: jax.Array,
):
    kT = jnp.swapaxes(A_k_cache, 2, 3).reshape(B * HD, SK)
    vT = jnp.swapaxes(A_v_cache, 2, 3).reshape(B * HD, SK)
    out = pl.pallas_call(
        _kernel,
        out_shape=jax.ShapeDtypeStruct((B, D), BF),
        in_specs=[pl.BlockSpec(memory_space=pl.ANY)] * 9,
        out_specs=pl.BlockSpec(memory_space=pltpu.VMEM),
        scratch_shapes=[
            pltpu.VMEM((B, D), BF),
            pltpu.VMEM((D,), BF),
            pltpu.VMEM((NSLOT, HD // 2, W), I32),
            pltpu.VMEM((NSLOT, HD // 2, W), I32),
            pltpu.VMEM((2, N_F32 * HR, W), F32),
            pltpu.VMEM((D // 2, HD), I32),
            pltpu.VMEM((HD // 2, D), I32),
            pltpu.VMEM((D // 2, F), I32),
            pltpu.VMEM((D // 2, F), I32),
            pltpu.VMEM((F // 2, D), I32),
            pltpu.VMEM((8, F), F32),
            pltpu.VMEM((8, F), F32),
            pltpu.VMEM((8, HD), F32),
            pltpu.SemaphoreType.DMA((7,)),
            pltpu.SemaphoreType.DMA((B, len(K_CHUNKS))),
            pltpu.SemaphoreType.DMA((B, len(V_CHUNKS))),
        ],
        compiler_params=pltpu.CompilerParams(vmem_limit_bytes=110 * 1024 * 1024),
    )(A_x.reshape(B, D), kT, vT, A_wq, A_wo, B_w_r, B_w_gate, B_w_up, B_w_down)
    return out.reshape(B, 1, D)
```
